```python
import os as _os
_os.environ.setdefault("JAX_PLATFORMS", "cpu")
import jax
import jax.numpy as jnp

def _softmax(x, axis=-1):
    return jax.nn.softmax(x, axis=axis)
def _gelu(x):
    return jax.nn.gelu(x, approximate=True)
def _silu(x):
    return jax.nn.silu(x)
def _sigmoid(x):
    return jax.nn.sigmoid(x)
def _layernorm(x, axis=-1, eps=1e-5):
    m = jnp.mean(x, axis=axis, keepdims=True)
    v = jnp.var(x, axis=axis, keepdims=True)
    return (x - m) / jnp.sqrt(v + eps)
def _scatter_add(tgt, idx, src, axis=0):
    return tgt.at[idx].add(src)
def _segment_sum(src, seg, n):
    return jax.ops.segment_sum(src, seg, n)
class _Rng:
    def __init__(self, key):
        self._k = key
    def _next(self):
        self._k, sub = jax.random.split(self._k)
        return sub
    def normal(self, shape):
        return jax.random.normal(self._next(), shape, dtype=jnp.bfloat16)
    def randint(self, lo, hi, shape):
        return jax.random.randint(self._next(), shape, lo, hi, dtype=jnp.int32)
    def uniform(self, shape, lo=0.0, hi=1.0):
        return jax.random.uniform(self._next(), shape, jnp.bfloat16, lo, hi)
    def permutation(self, n):
        return jax.random.permutation(self._next(), n)


kernel_name = 'concat_heads__ssm_conv_s4__sliding_local_dilated__prompt'

def setup_inputs():
    _rng = _Rng(jax.random.key(int.from_bytes(__import__("os").urandom(4), "little")))
    _w = (lambda a: (lambda t: t.astype(jnp.bfloat16) if jnp.issubdtype(t.dtype, jnp.floating) else t)(jnp.asarray(a)))
    def _A_setup():
        B, L, D, N = 1, 2048, 640, 192
        A_re = -jnp.exp((lambda *s: _rng.normal(s) * 0.8)(D, N))
        A_im = jnp.pi * (lambda *s: _rng.normal(s) * 0.8)(D, N)
        B_re = (lambda *s: _rng.normal(s) * 0.8)(D, N)
        B_im = (lambda *s: _rng.normal(s) * 0.8)(D, N)
        C_re = (lambda *s: _rng.normal(s) * 0.8)(D, N)
        C_im = (lambda *s: _rng.normal(s) * 0.8)(D, N)
        log_dt = (lambda *s: _rng.normal(s) * 0.8)(D) * 0.5 - 4.0
        Dskip = (lambda *s: _rng.normal(s) * 0.05)(D)
        return {
            "u": _w((lambda *s: _rng.normal(s) * 0.05)(B, L, D)),
            "A_re": _w(A_re),
            "A_im": _w(A_im),
            "B_re": _w(B_re),
            "B_im": _w(B_im),
            "C_re": _w(C_re),
            "C_im": _w(C_im),
            "log_dt": _w(log_dt),
            "Dskip": _w(Dskip),
        }
    _A_in = _A_setup()

    def _B_setup():
        B, S, D = 1, 2048, 640
        return {
            "x": _w((lambda *s: _rng.normal(s) * 0.2)(B, S, D)),
            "wqkv": _w((lambda *s: _rng.normal(s) * 0.2)(D, 3 * D)),
            "wo": _w((lambda *s: _rng.normal(s) * 0.05)(D, D)),
        }
    _B_in = _B_setup()

    return {
        "A_u": _A_in["u"],
        "A_A_re": _A_in["A_re"],
        "A_A_im": _A_in["A_im"],
        "A_B_re": _A_in["B_re"],
        "A_B_im": _A_in["B_im"],
        "A_C_re": _A_in["C_re"],
        "A_C_im": _A_in["C_im"],
        "A_log_dt": _A_in["log_dt"],
        "A_Dskip": _A_in["Dskip"],
        "B_x": _B_in["x"],
        "B_wqkv": _B_in["wqkv"],
        "B_wo": _B_in["wo"],
    }

def reference(A_u, A_A_re, A_A_im, A_B_re, A_B_im, A_C_re, A_C_im, A_log_dt, A_Dskip, B_x, B_wqkv, B_wo):
    def _A_ref(u, A_re, A_im, B_re, B_im, C_re, C_im, log_dt, Dskip):
        Bsz, L, D = u.shape
        dt = jnp.exp(log_dt)[:, None]
        A = A_re + 1j * A_im
        Bc = B_re + 1j * B_im
        Cc = C_re + 1j * C_im
        logdA = dt * A
        dB = dt * Bc
        l = (lambda x, dt: x.astype(dt))(jnp.arange(L), A_re.dtype)
        P = jnp.exp(logdA[:, :, None] * l[None, None, :])
        K = jnp.einsum("dn,dnl,dn->dl", Cc, P, dB).real
        L2 = 2 * L
        Kp = jnp.pad(K, ((0, 0), (0, L)))
        up = (lambda x, *d: x.transpose(*d))(u, 0, 2, 1)
        up = jnp.pad(up, ((0, 0), (0, 0), (0, L)))
        Kf = (lambda x, axes=(-2,-1): jnp.fft.rfft2(x.astype(jnp.float32), axes=axes))(Kp[:, None, :], axes=(-2, -1))
        Uf = (lambda x, axes=(-2,-1): jnp.fft.rfft2(x.astype(jnp.float32), axes=axes))(up[:, :, None, :], axes=(-2, -1))
        Yf = Uf * Kf[None, :, :, :]
        y = (lambda x, s, axes=(-2,-1): jnp.fft.irfft2(x, s=s, axes=axes).astype(jnp.bfloat16))(Yf, (1, L2), axes=(-2, -1))[:, :, 0, :L]
        y = (lambda x, *d: x.transpose(*d))(y, 0, 2, 1) + u * Dskip[None, None, :]
        return y

    def _B_ref(x, wqkv, wo):
        B, S, D = x.shape
        H = 32; Dh = D // H
        W, dil = 8, 2
        qkv = (lambda x, *d: x.transpose(*d))((x @ wqkv).reshape(B, S, 3, H, Dh), 2, 0, 3, 1, 4)
        q, k, v = qkv[0], qkv[1], qkv[2]
        scale = Dh ** -0.5
        pos = jnp.arange(S)
        off = jnp.arange(W) * dil
        idx = pos[:, None] - off[None, :]
        mask = idx >= 0
        idx_c = jnp.where(mask, idx, 0).reshape(-1)
        kg = k[:, :, idx_c, :].reshape(B, H, S, W, Dh)
        vg = v[:, :, idx_c, :].reshape(B, H, S, W, Dh)
        logits = jnp.einsum("bhsd,bhswd->bhsw", q, kg) * scale
        logits = jnp.where(mask[None, None, :, :], logits, -1e9)
        attn = _softmax(logits, axis=-1)
        o = jnp.einsum("bhsw,bhswd->bhsd", attn, vg)
        return (lambda x, *d: x.transpose(*d))(o, 0, 2, 1, 3).reshape(B, S, D) @ wo

    a = _A_ref(A_u, A_A_re, A_A_im, A_B_re, A_B_im, A_C_re, A_C_im, A_log_dt, A_Dskip)
    b = _B_ref(B_x, B_wqkv, B_wo)
    return jnp.concatenate([a, b], axis=-1)
```

```python
import jax
import jax.numpy as jnp
import numpy as np
from jax import lax
import jax.experimental.pallas as pl
import jax.experimental.pallas.tpu as pltpu

L = 2048
D = 640
N = 192
H, DH = 32, 20
WIN, DIL = 8, 2
C = 128
NC = L // C
DT = D // 128
RB = 128
NB = L // RB
HALO = 16
F32 = jnp.float32
BF16 = jnp.bfloat16

L1 = ((1, 5), (2, 6), (3, 7), (4, 8), (258, 516), (260, 520), (262, 772), (264, 776), (1032, 1288), (1544, 1800))
L1_STEPS = ((1, 2), (3, 4), (5, 6), (7, 8), (258, 260, 262), (264, 516, 520), (772, 776, 1032), (1288, 1544, 1800))
CHUNK_BLOCK = (0, 1, 2, 3, 4, 5, 5, 5, 6, 7, 7, 7, 7, 7, 7, 7)


def _round_bf16(l):
    if l < 256:
        return l
    s = 1 << (l.bit_length() - 8)
    q, r = divmod(l, s)
    if 2 * r > s or (2 * r == s and q % 2 == 1):
        q += 1
    return q * s


def _row_pairs(a):
    bits = a.astype(BF16).view(np.uint16).astype(np.uint32)
    return (bits[..., 0::2, :] | (bits[..., 1::2, :] << 16)).view(np.int32)


def _dft_tables():
    row = np.arange(2 * C)
    part = (row // 8) % 2
    theta = 2.0 * np.pi * (8 * (row // 16) + row % 8 + 0.5) / (2 * C)

    def fwd(j):
        a = theta[:, None] * np.asarray(j, np.float64)[None, :]
        return np.where(part[:, None] == 0, np.cos(a), -np.sin(a))

    fu = np.stack([fwd(C * m + np.arange(C)) for m in range(4)])
    lane = np.arange(128)
    h, p, j = (lane // 8) % 2, (lane // 2) % 4, 2 * (lane // 16) + lane % 2
    l1 = np.asarray(L1)
    v = [l1[4 * (i // 2) + p, i % 2] + 8 * (16 * h + j) for i in range(4)] + [l1[8 + p % 2, p // 2] + 8 * (16 * h + j)]
    last = lane == 127
    blocks = [l1[p, h] + 8 * j, l1[p, h] + 8 * (16 + j),
              np.where(last, v[1], v[2]), v[2], np.where(last, v[2], v[3]), v[3],
              np.where(last, v[3], v[4]), v[4]]
    fk = np.zeros((NC, 2 * C, 128))
    for m in range(NC):
        for l in range(C * m + 1, min(C * m + C, L - 1) + 1):
            at = np.nonzero(blocks[CHUNK_BLOCK[m]] == _round_bf16(l))[0][0]
            fk[m, :, at] += fwd([l])[:, 0]
    inv = fu[:, 16 * (row // 16) + 8 * (row % 2) + (row // 2) % 8].transpose(0, 2, 1) / C
    return _row_pairs(np.concatenate([fu, fk])), _row_pairs(inv)


_FWD, _INV = _dft_tables()


def _iota(dim, shape=(8, 128)):
    return lax.broadcasted_iota(jnp.int32, shape, dim)


def _rows(start, size):
    return pl.ds(start if isinstance(start, int) else pl.multiple_of(start, min(size, 16)), size)


def _cmul(a, b):
    return a[0] * b[0] - a[1] * b[1], a[0] * b[1] + a[1] * b[0]


def _cmul_conj(a, b):
    return a[0] * b[0] + a[1] * b[1], a[1] * b[0] - a[0] * b[1]


def _csqr(a):
    t = a[0] * a[1]
    return a[0] * a[0] - a[1] * a[1], t + t


def _pack(a, b):
    return pltpu.bitcast(jnp.concatenate([a, b], axis=0).astype(BF16), jnp.int32)


def _zip(a, b):
    return lax.bitcast_convert_type(pltpu.pack_elementwise([a, b], packed_dtype=BF16), jnp.int32)


def _bf(a):
    return pltpu.bitcast(a, BF16)


def _dot(a, b):
    return jnp.dot(a, b, preferred_element_type=F32)


def _dot_nt(a, b):
    return lax.dot_general(a, b, (((1,), (1,)), ((), ())), preferred_element_type=F32)


def _multipliers(z1):
    lo = _iota(0) < 4
    z = {1: z1}
    for s in range(8):
        z[2 << s] = _csqr(z[1 << s])
    z8r = [pltpu.roll(t, 4, 0) for t in z[8]]
    out = list(z[256])
    for half, top in enumerate(([pltpu.roll(t, 4, 0) for t in z[128]], z[128])):
        out += [jnp.where(lo, a, b) if half == 0 else jnp.where(lo, b, a) for a, b in zip(z[8], z8r)]
        out += [jnp.where(lo, 1.0, top[0]), jnp.where(lo, 0.0, top[1])]
    return out


def _factor_tables(g, zw_ref, lhs_ref, rhs_ref):
    lo64, lo = _iota(1) < 64, _iota(0) < 4
    for part, grp in ((0, 0), (0, 1), (1, 0)):
        def load(a):
            return [zw_ref[2 * a + c, part, _rows(16 * g + 8 * grp, 8), :] for c in range(2)]

        def columns(a, b):
            re, im = _zip(a[0], b[0]), _zip(a[1], b[1])
            if part == 0:
                return (grp, 0, re), (grp, 1, im)
            return ((0, 2, jnp.where(lo64, re, pltpu.roll(im, 64, 1))),
                    (1, 2, jnp.where(lo64, pltpu.roll(re, 64, 1), im)))

        x, y, held = [None, None], {}, {}
        for k in range(8):
            yield "table", (48 if part == 0 else 54), x[1] and x[1][0]
            for half in range(2):
                ratio = load(3 + 2 * half)
                even = load(4 + 2 * half) if k == 0 else _cmul(x[half], ratio)
                x[half] = _cmul(even, ratio)
                for to, col, val in columns(even, x[half]):
                    rhs_ref[4 * g + 2 * to + half, 8 * k:8 * k + 8, 128 * col:128 * col + 128] = val
            if k == 0:
                w = load(1)
                y[0] = (w[0], -w[1])
            ratio, back = (load(0), 1) if k < 4 else (load(2), 256)
            for l in L1_STEPS[k]:
                y[l] = _cmul_conj(y[l - back], ratio)
            for q, (la, lb) in enumerate(L1):
                if lb not in L1_STEPS[k]:
                    continue
                held[q] = columns(y[la], y[lb])
                if q >= 5:
                    for (to, col, a), (_, _, b) in zip(held[q - 5], held[q]):
                        b = pltpu.roll(b, 4, 0)
                        at = slice(8 * q - 40, 8 * q - 32), slice(128 * col, 128 * col + 128)
                        lhs_ref[(4 * g + 2 * to,) + at] = jnp.where(lo, a, b)
                        lhs_ref[(4 * g + 2 * to + 1,) + at] = jnp.where(lo, b, a)


def _kernel_values(g, lhs_ref, rhs_ref, tmp_ref, kd_ref):
    lane = _iota(1)
    pick = (lane & ~6) | (_iota(0) & 6)
    bit2, bit4, bit8, last = (lane & 2) != 0, (lane & 4) != 0, (lane & 8) != 0, lane == 127
    for quad in range(4):
        yield "values"
        o = _dot_nt(_bf(lhs_ref[4 * g + quad]), _bf(rhs_ref[4 * g + quad]))
        m = [None] * 10
        for r in range(10):
            m[r // 2 + 5 * ((r + quad) % 2)] = jnp.take_along_axis(o[8 * r:8 * r + 8], pick, axis=1)
            if r % 4 == 1:
                yield o[8 * r:8 * r + 8]
        m = [jnp.where(bit2, m[2 * i + 1], m[2 * i]) for i in range(5)]
        for i, val in enumerate((jnp.where(bit4, m[1], m[0]), jnp.where(bit4, m[3], m[2]), m[4])):
            tmp_ref[i, 8 * quad:8 * quad + 8, :] = val
    v = [_zip(*[tmp_ref[i // 2, pl.ds(2 * c + i % 2, 8, stride=4), :] for c in range(2)]) for i in range(6)]
    v[4] = jnp.where(bit4, v[5], v[4])
    blocks = [jnp.where(bit8, pltpu.roll(v[1], 8, 1), v[0]), jnp.where(bit8, v[1], pltpu.roll(v[0], 120, 1)),
              jnp.where(last, v[1], v[2]), v[2], jnp.where(last, v[2], v[3]), v[3],
              jnp.where(last, v[3], v[4]), v[4]]
    for b in range(8):
        kd_ref[b, _rows(8 * g, 8), :] = blocks[b]


def _chunk_products(q, t, uf_ref, kf_ref, yf_ref):
    cols = slice(128 * t, 128 * t + 128)

    def load(ref, m):
        re, im = ref[m, _rows(16 * q, 8), cols], ref[m, _rows(16 * q + 8, 8), cols]
        return re, im, re + im

    prev = None
    for i0 in range(0, NC, 4):
        acc, win = [None] * 4, {}
        for m in range(i0 + 4):
            yield "conv", 6 * min(4, i0 + 4 - m) + 4
            k = load(kf_ref, m)
            for a in range(4):
                j = i0 + a - m
                if j < 0:
                    continue
                if j not in win:
                    win[j] = load(uf_ref, j)
                p = [s * u for s, u in zip(k, win[j])]
                acc[a] = p if acc[a] is None else [s + u for s, u in zip(acc[a], p)]
        for a in range(4):
            z = acc[a][0] - acc[a][1], acc[a][2] - acc[a][0] - acc[a][1]
            y = z if prev is None else (z[0] + prev[0], z[1] + prev[1])
            prev = z
            yf_ref[i0 + a, _rows(8 * q, 8), cols] = _zip(*y)


def _scores(row, qkv, prob):
    lane = _iota(1)
    even, lo64 = (lane & 32) == 0, lane < 64

    def fold(a, b, mask, shift):
        return jnp.where(mask, a, b) + pltpu.roll(jnp.where(mask, b, a), shift, 1)

    def total(terms):
        return ((terms[0] + terms[1]) + (terms[2] + terms[3])) + terms[4]

    half = []
    for pair in range(2):
        at = HALO + row + 16 * pair
        q, two = None, [None] * WIN
        for w in range(WIN // 2):
            yield "attn", 48
            q = q or [[qkv[t][_rows(at + 8 * g, 8), :] for t in range(DT)] for g in range(2)]
            k = [[qkv[DT + t][pl.ds(at - DIL * w + 8 * g, 8), :] for t in range(DT)] for g in (-1, 0, 1)]
            for far in range(2):
                first, last = [total([a * b for a, b in zip(q[g], k[g + 1 - far])]) for g in range(2)]
                x = fold(first, last, even, 32)
                two[w + 4 * far] = fold(half[0][w + 4 * far], x, lo64, 64) if pair else x
        half.append(two)
    logit = [x * (DH ** -0.5) for x in half[1]]
    if isinstance(row, int) and row < DIL * (WIN - 1):
        logit = [jnp.where(row + 8 * (lane >> 5) + _iota(0) - DIL * w >= 0, x, -1e9) for w, x in enumerate(logit)]
    yield "attn", 45
    mx = logit[0]
    for x in logit[1:]:
        mx = jnp.maximum(mx, x)
    e = [jnp.exp(x - mx) for x in logit]
    inv = 1.0 / (((e[0] + e[1]) + (e[2] + e[3])) + ((e[4] + e[5]) + (e[6] + e[7])))
    prob.extend(x * inv for x in e)


def _mix(row, o_row, qkv, prob, o_ref):
    head = _iota(1) & 31
    for pair in range(2):
        at = HALO + row + 16 * pair
        out = [None, None]
        for w in range(WIN // 2):
            yield "attn", 42
            v = [[qkv[2 * DT + t][pl.ds(at - DIL * w + 8 * g, 8), :] for t in range(DT)] for g in (-1, 0, 1)]
            for far in range(2):
                both = prob[w + 4 * far]
                for g in range(2):
                    p = jnp.take_along_axis(both, head + 32 * (2 * pair + g), axis=1)
                    terms = [p * x for x in v[g + 1 - far]]
                    out[g] = terms if out[g] is None else [s + u for s, u in zip(out[g], terms)]
        for t in range(DT):
            o_ref[_rows(o_row + 8 * pair, 8), 128 * t:128 * t + 128] = _pack(out[0][t], out[1][t])


def _interleave(slots, n_slots, work, total, gates, lead, ahead):
    done, pending, i, queue = 0, next(work, None), lead - 1, [None] * ahead
    for item in _chain(slots, [None] * ahead):
        if isinstance(item, str):
            if pending is not None and pending[2] is not None:
                gates[item](pltpu.bitcast(pending[2], jnp.int32))
            continue
        queue.append(item)
        token, gated, i = queue.pop(0), (), i + 1
        token = token() if callable(token) else token
        while pending is not None and done * n_slots < total * i:
            if token is not None and pending[0] not in gated:
                gates[pending[0]](token)
                gated = gated + (pending[0],)
            done += pending[1]
            pending = next(work, None)
    for _ in work:
        pass


def _chain(*gens):
    for g in gens:
        yield from g


def _kernel(u_hbm, are_hbm, aim_hbm, bre_hbm, bim_hbm, cre_hbm, cim_hbm, ldt_hbm, skip_hbm,
            x_hbm, w_hbm, wo_hbm, fwd_hbm, inv_hbm, out_hbm,
            ldt_ref, skip_ref, par_ref, turn_ref, direct_ref, zw_ref,
            lhs_ref, rhs_ref, tmp_ref, kd_ref,
            u_ref, x_ref, w_ref, wo_ref, fwd_ref, inv_ref, xp_ref, wp_ref, wof_ref, wop_ref,
            uf_ref, kf_ref, yf_ref, qkv_ref, o_ref, ya_ref, yb_ref,
            zero_ref, isem, asem, bsem):
    zero_ref[0] = 0

    srcs = (ldt_hbm, aim_hbm, skip_hbm, are_hbm, bre_hbm, bim_hbm, cre_hbm, cim_hbm,
            u_hbm, fwd_hbm, w_hbm, x_hbm, wo_hbm, inv_hbm)
    dsts = (ldt_ref, par_ref.at[1], skip_ref, *[par_ref.at[j] for j in (0, 2, 3, 4, 5)],
            u_ref, fwd_ref, w_ref, x_ref, wo_ref, inv_ref)
    loads = [pltpu.make_async_copy(s, d, isem.at[i]) for i, (s, d) in enumerate(zip(srcs, dsts))]

    def arrive(done, begin):
        for c in done:
            c.wait()
        for c in begin:
            c.start()

    arrive((), loads[0:2])
    arrive(loads[0:2], loads[2:8])
    dt = jnp.exp(ldt_ref[...].astype(F32)).astype(BF16).astype(F32).reshape(1, D)

    @pl.loop(0, 2)
    def _(i):
        for r in range(0, N // 2, 16):
            rows = _rows(N // 2 * i + r, 16)
            angle = dt * par_ref[1, rows, :].astype(F32)
            turn_ref[0, rows, :] = jnp.cos(angle)
            turn_ref[1, rows, :] = jnp.sin(angle)

    arrive(loads[2:8], loads[8:10])
    skip = skip_ref[...].astype(F32).reshape(1, D)
    for t in range(DT):
        cols = slice(128 * t, 128 * t + 128)
        are, bre, bim, cre, cim = [par_ref[j, :, cols].astype(F32) for j in (0, 2, 3, 4, 5)]
        h = dt[:, cols]
        e = jnp.exp(h * are)
        w = _cmul((cre, cim), (h * bre, h * bim))
        direct_ref[:, cols] = jnp.sum(w[0], axis=0, keepdims=True) + skip[:, cols]
        vals = e * turn_ref[0, :, cols], e * turn_ref[1, :, cols], w[0], w[1]
        for part in range(2):
            tr = [(v[0:128] if part == 0 else
                   jnp.concatenate([v[128:N], pltpu.roll(v[128:N], 120, 1)], axis=0)).T for v in vals]
            for r in range(0, 128, 8 + 8 * part):
                row = [v[r:r + 8] for v in tr]
                for a, v in enumerate(row + _multipliers(row[:2])):
                    zw_ref[a, part, 128 * t + r:128 * t + r + 8, :] = v

    def permute_weights(i):
        lane = _iota(1)
        res = lane - 5 * ((lane * 205) >> 10)
        for t in range(DT):
            idx = (DH * (lane & 31) + 5 * (lane >> 5) + t) & 127
            for r in range(D // 32):
                rows = pl.ds(D // 2 * i + 16 * r, 16)
                for p in range(3):
                    acc = None
                    for s in range(DT):
                        c0 = D * p + 128 * s
                        x = pltpu.bitcast(w_ref[rows, c0:c0 + 128], jnp.int32)
                        acc = x if acc is None else jnp.where(res == (t - 3 * s) % 5, x, acc)
                    c0 = D * p + 128 * t
                    wp_ref[_rows(D // 4 * i + 8 * r, 8), c0:c0 + 128] = jnp.take_along_axis(acc, idx, axis=1)

    def transform_u(m):
        for t in range(DT):
            cols = slice(128 * t, 128 * t + 128)
            r = _dot(_bf(fwd_ref[m & 3]), u_ref[_rows(m * C, C), cols])
            uf_ref[m, 0:2 * C, cols] = r
            for i in range(0, 2 * C, 128):
                yield r[i:i + 8]

    def kernel_step(values, tables, chunks):
        spare = _rows(zero_ref[0], 8)

        def gate(token):
            zw_ref[14, 0, spare, :] = token

        def gate_values(token):
            rhs_ref[D // 4, spare, 0:128] = token

        slots = []
        for j, g in enumerate(values):
            slots.append(_kernel_values(g, lhs_ref, rhs_ref, tmp_ref.at[j], kd_ref))
            if chunks and j % 2:
                slots.append(transform_u(chunks[j // 2]))
        work = [_factor_tables(g, zw_ref, lhs_ref, rhs_ref) for g in tables]
        _interleave(_chain(*slots), 18 * len(tables) + 16, _chain(*work), 1200 * len(tables),
                    {"table": gate, "values": gate_values}, 1, 24)

    kernel_step((), (0, 1), ())

    @pl.loop(0, 4)
    def _(i):
        kernel_step((2 * i, 2 * i + 1), (2 * i + 2, 2 * i + 3), ())

    arrive(loads[8:10], loads[10:14])

    @pl.loop(4, D // 32 - 1)
    def _(i):
        kernel_step((2 * i, 2 * i + 1), (2 * i + 2, 2 * i + 3), (i - 4,))

    def repack_x(b):
        xp_ref[_rows(RB // 2 * b, RB // 2), :] = pltpu.bitcast(x_ref[_rows(RB * b, RB), :], jnp.int32)

    arrive(loads[10:14], ())
    kernel_step((D // 16 - 2, D // 16 - 1), (), (NC - 1,))
    for i in range(2):
        permute_weights(i)
    for t in range(DT):
        cols = slice(128 * t, 128 * t + 128)
        for m in range(NC):
            kf_ref[m, 0:2 * C, cols] = _dot_nt(_bf(fwd_ref[m + 4]), _bf(kd_ref[CHUNK_BLOCK[m], 64 * t:64 * t + 64, :]))
        wof_ref[t] = wo_ref[:, cols].astype(F32)
        for dh in range(DH):
            at = 64 * (dh % 5) + 16 * (dh // 5)
            wop_ref[at:at + 16, cols] = pltpu.bitcast(wof_ref[t, pl.ds(dh, H, stride=DH), :].astype(BF16), jnp.int32)
    for b in range(3):
        repack_x(b)

    def block_rows(b):
        return _rows(RB * b, RB)

    def a_copy(b):
        return pltpu.make_async_copy(ya_ref.at[block_rows(b)], out_hbm.at[block_rows(b), pl.ds(0, D)], asem.at[b])

    def b_copy(b):
        return pltpu.make_async_copy(yb_ref.at[block_rows(b)], out_hbm.at[block_rows(b), pl.ds(D, D)], bsem.at[b])

    qkv = [qkv_ref.at[c] for c in range(3 * DT)]

    def project(b):
        for c in range(3 * DT):
            r = _dot(_bf(xp_ref[_rows(RB // 2 * b, RB // 2), :]), _bf(wp_ref[:, 128 * c:128 * c + 128]))
            for i in range(0, RB, 16):
                def piece(c=c, i=i, r=r):
                    qkv[c][_rows(HALO + RB * b + i, 16), :] = r[i:i + 16]
                    return r[i + 8:i + 16]
                yield piece

    def out_project(b):
        for t in range(DT):
            cols = slice(128 * t, 128 * t + 128)
            r = _dot(_bf(o_ref[_rows(RB // 2 * b, RB // 2), :]), _bf(wop_ref[:, cols]))
            for i in range(0, RB, 8):
                yb_ref[_rows(RB * b + i, 8), cols] = r[i:i + 8].astype(BF16)
            for i in range(0, RB, 16):
                yield r[i + 8:i + 16]

    def inverse(b):
        for t in range(DT):
            cols = slice(128 * t, 128 * t + 128)
            r = _dot(_bf(inv_ref[b & 3]), _bf(yf_ref[b, :, cols]))
            rows = block_rows(b)
            ya_ref[rows, cols] = (r + u_ref[rows, cols].astype(F32) * direct_ref[:, cols]).astype(BF16)
            for i in range(0, RB, 16):
                yield r[i + 8:i + 16]

    def vector_work(columns, b_attn):
        conv = _chain(*[_chunk_products(q, t, uf_ref, kf_ref, yf_ref) for q, t in columns])
        prob = [[] for _ in range(4)]
        for g in range(5 * (b_attn is not None)):
            for _, item in zip(range(len(columns) * (8 if g else 5)), conv):
                yield item
            parts = []
            if g > 0:
                parts.append(_mix(RB * b_attn + 32 * g - 32, RB // 2 * b_attn + 16 * g - 16, qkv, prob[g - 1], o_ref))
            if g < 4:
                parts.insert(len(parts) if columns else 0, _scores(RB * b_attn + 32 * g, qkv, prob[g]))
            yield from _chain(*parts)
        yield from conv

    def step(slots, n_slots, *work):
        spare = _rows(zero_ref[0], 8)

        def gate_conv(token):
            kf_ref[NC, spare, 0:128] = token

        def gate_attn(token):
            qkv_ref[3 * DT, spare, :] = token

        total = sum(len(columns) * 976 + (b is not None) * 4 * 765 for columns, b in work)
        _interleave(slots, n_slots, _chain(*[vector_work(*w) for w in work]), total,
                    {"conv": gate_conv, "attn": gate_attn}, 10, 1)

    def region(f):
        pl.when(zero_ref[0] == 0)(f)

    columns = [(q, t) for q in range(NC) for t in range(DT)]

    def take(n):
        return [columns.pop(0) for _ in range(n)]

    region(lambda: step(project(0), 124, (take(9), None)))
    for c in range(DT, 3 * DT):
        qkv[c][0:HALO, :] = jnp.broadcast_to(qkv[c][HALO:HALO + 1, :], (HALO, 128))
    region(lambda: step(project(1), 124, (take(4), 0)))

    for b in range(2, NB - 2, 2):
        @region
        def _():
            repack_x(b + 1)
            step(_chain(out_project(b - 2), project(b), project(b + 1), out_project(b - 1)), 325,
                 (take(5), b - 1), (take(5 + (b == 2)), b))
            repack_x(b + 2)
            arrive((), [b_copy(b - 2), b_copy(b - 1)])

    @region
    def _():
        step(_chain(out_project(NB - 4), project(NB - 2)), 165, (take(6), NB - 3))
        repack_x(NB - 1)
        b_copy(NB - 4).start()

    def inverses(blocks):
        return _chain(*[inverse(b) for b in blocks])

    last = NB - 1
    step(_chain(inverses(range(0, 4)), out_project(last - 2)), 100, ([], last - 1))
    arrive((), [b_copy(last - 2)] + [a_copy(b) for b in range(0, 4)])
    for blocks in (range(4, 8), range(8, 12)):
        for _ in inverses(blocks):
            pass
        arrive((), [a_copy(b) for b in blocks])
    for piece in project(last):
        piece()
    for _ in out_project(last - 1):
        pass
    b_copy(last - 1).start()
    step(inverses(range(12, 16)), 70, ([], last))
    arrive((), [a_copy(b) for b in range(12, 16)])
    for _ in out_project(last):
        pass
    b_copy(last).start()
    for b in range(NB):
        a_copy(b).wait()
        b_copy(b).wait()


@jax.jit
def pallas_concat_heads__ssm_conv_s4__sliding_local_dilated__prompt_kernel(
    A_u: jax.Array,
    A_A_re: jax.Array,
    A_A_im: jax.Array,
    A_B_re: jax.Array,
    A_B_im: jax.Array,
    A_C_re: jax.Array,
    A_C_im: jax.Array,
    A_log_dt: jax.Array,
    A_Dskip: jax.Array,
    B_x: jax.Array,
    B_wqkv: jax.Array,
    B_wo: jax.Array,
):
    hbm = pl.BlockSpec(memory_space=pl.ANY)
    V = pltpu.VMEM
    I32 = jnp.int32
    scratch = (
        [V((D,), BF16), V((D,), BF16), V((6, N, D), BF16), V((2, N, D), F32), V((1, D), F32), V((15, 2, D, 128), F32)]
        + [V((D // 4, 40, 2 * N), I32), V((D // 4 + 1, 64, 2 * N), I32), V((2, 3, 32, 128), F32), V((8, D // 2, 128), I32)]
        + [V((L, D), BF16), V((L, D), BF16), V((D, 3 * D), BF16), V((D, D), BF16),
           V(_FWD.shape, I32), V(_INV.shape, I32),
           V((L // 2, D), I32), V((D // 2, 3 * D), I32), V((DT, D, 128), F32), V((D // 2, D), I32),
           V((NC, 2 * C + 8, D), F32), V((NC + 1, 2 * C + 24, D), F32), V((NC, C, D), I32),
           V((3 * DT + 1, HALO + L + 8, 128), F32), V((L // 2, D), I32)]
        + [V((L, D), BF16)] * 2 + [pltpu.SMEM((1,), I32)]
        + [pltpu.SemaphoreType.DMA((14,))]
        + [pltpu.SemaphoreType.DMA((NB,))] * 2
    )
    out = pl.pallas_call(
        _kernel,
        out_shape=jax.ShapeDtypeStruct((L, 2 * D), BF16),
        in_specs=[hbm] * 14,
        out_specs=hbm,
        scratch_shapes=scratch,
        compiler_params=pltpu.CompilerParams(vmem_limit_bytes=120 * 1024 * 1024),
    )(A_u.reshape(L, D), A_A_re.T, A_A_im.T, A_B_re.T, A_B_im.T, A_C_re.T, A_C_im.T,
      A_log_dt, A_Dskip, B_x.reshape(L, D), B_wqkv, B_wo, _FWD, _INV)
    return out.reshape(1, L, 2 * D)
```

```python
import jax
import jax.numpy as jnp
import numpy as np
from jax import lax
import jax.experimental.pallas as pl
import jax.experimental.pallas.tpu as pltpu

L = 2048
D = 640
N = 192
H, DH = 32, 20
WIN, DIL = 8, 2
C = 128
NC = L // C
DT = D // 128
RB = 128
NB = L // RB
HALO = 16
F32 = jnp.float32
BF16 = jnp.bfloat16

L1 = ((1, 5), (2, 6), (3, 7), (4, 8), (258, 516), (260, 520), (262, 772), (264, 776), (1032, 1288), (1544, 1800))
L1_STEPS = ((1, 2), (3, 4), (5, 6), (7, 8), (258, 260, 262), (264, 516, 520), (772, 776, 1032), (1288, 1544, 1800))
CHUNK_BLOCK = (0, 1, 2, 3, 4, 5, 5, 5, 6, 7, 7, 7, 7, 7, 7, 7)


def _round_bf16(l):
    if l < 256:
        return l
    s = 1 << (l.bit_length() - 8)
    q, r = divmod(l, s)
    if 2 * r > s or (2 * r == s and q % 2 == 1):
        q += 1
    return q * s


def _row_pairs(a):
    bits = a.astype(BF16).view(np.uint16).astype(np.uint32)
    return (bits[..., 0::2, :] | (bits[..., 1::2, :] << 16)).view(np.int32)


def _dft_tables():
    row = np.arange(2 * C)
    part = (row // 8) % 2
    theta = 2.0 * np.pi * (8 * (row // 16) + row % 8 + 0.5) / (2 * C)

    def fwd(j):
        a = theta[:, None] * np.asarray(j, np.float64)[None, :]
        return np.where(part[:, None] == 0, np.cos(a), -np.sin(a))

    fu = np.stack([fwd(C * m + np.arange(C)) for m in range(4)])
    lane = np.arange(128)
    h, p, j = (lane // 8) % 2, (lane // 2) % 4, 2 * (lane // 16) + lane % 2
    l1 = np.asarray(L1)
    v = [l1[4 * (i // 2) + p, i % 2] + 8 * (16 * h + j) for i in range(4)] + [l1[8 + p % 2, p // 2] + 8 * (16 * h + j)]
    last = lane == 127
    blocks = [l1[p, h] + 8 * j, l1[p, h] + 8 * (16 + j),
              np.where(last, v[1], v[2]), v[2], np.where(last, v[2], v[3]), v[3],
              np.where(last, v[3], v[4]), v[4]]
    fk = np.zeros((NC, 2 * C, 128))
    for m in range(NC):
        for l in range(C * m + 1, min(C * m + C, L - 1) + 1):
            at = np.nonzero(blocks[CHUNK_BLOCK[m]] == _round_bf16(l))[0][0]
            fk[m, :, at] += fwd([l])[:, 0]
    inv = fu[:, 16 * (row // 16) + 8 * (row % 2) + (row // 2) % 8].transpose(0, 2, 1) / C
    return _row_pairs(np.concatenate([fu, fk])), _row_pairs(inv)


_FWD, _INV = _dft_tables()


def _iota(dim, shape=(8, 128)):
    return lax.broadcasted_iota(jnp.int32, shape, dim)


def _rows(start, size):
    return pl.ds(start if isinstance(start, int) else pl.multiple_of(start, min(size, 16)), size)


def _cmul(a, b):
    return a[0] * b[0] - a[1] * b[1], a[0] * b[1] + a[1] * b[0]


def _cmul_conj(a, b):
    return a[0] * b[0] + a[1] * b[1], a[1] * b[0] - a[0] * b[1]


def _csqr(a):
    t = a[0] * a[1]
    return a[0] * a[0] - a[1] * a[1], t + t


def _pack(a, b):
    return pltpu.bitcast(jnp.concatenate([a, b], axis=0).astype(BF16), jnp.int32)


def _zip(a, b):
    return lax.bitcast_convert_type(pltpu.pack_elementwise([a, b], packed_dtype=BF16), jnp.int32)


def _bf(a):
    return pltpu.bitcast(a, BF16)


def _dot(a, b):
    return jnp.dot(a, b, preferred_element_type=F32)


def _dot_nt(a, b):
    return lax.dot_general(a, b, (((1,), (1,)), ((), ())), preferred_element_type=F32)


def _multipliers(z1):
    lo = _iota(0) < 4
    z = {1: z1}
    for s in range(8):
        z[2 << s] = _csqr(z[1 << s])
    z8r = [pltpu.roll(t, 4, 0) for t in z[8]]
    out = list(z[256])
    for half, top in enumerate(([pltpu.roll(t, 4, 0) for t in z[128]], z[128])):
        out += [jnp.where(lo, a, b) if half == 0 else jnp.where(lo, b, a) for a, b in zip(z[8], z8r)]
        out += [jnp.where(lo, 1.0, top[0]), jnp.where(lo, 0.0, top[1])]
    return out


def _factor_tables(g, zw_ref, lhs_ref, rhs_ref):
    lo64, lo = _iota(1) < 64, _iota(0) < 4
    for part, grp in ((0, 0), (0, 1), (1, 0)):
        def load(a):
            return [zw_ref[2 * a + c, part, _rows(16 * g + 8 * grp, 8), :] for c in range(2)]

        def columns(a, b):
            re, im = _zip(a[0], b[0]), _zip(a[1], b[1])
            if part == 0:
                return (grp, 0, re), (grp, 1, im)
            return ((0, 2, jnp.where(lo64, re, pltpu.roll(im, 64, 1))),
                    (1, 2, jnp.where(lo64, pltpu.roll(re, 64, 1), im)))

        x, y, held, ratio = [None, None], {}, {}, {}
        for k in range(8):
            yield "table", (48 if part == 0 else 54), x[1] and x[1][0]
            for half in range(2):
                if k == 0 or half == 1:
                    ratio[half] = load(3 + 2 * half)
                even = load(4 + 2 * half) if k == 0 else _cmul(x[half], ratio[half])
                x[half] = _cmul(even, ratio[half])
                for to, col, val in columns(even, x[half]):
                    rhs_ref[4 * g + 2 * to + half, 8 * k:8 * k + 8, 128 * col:128 * col + 128] = val
            if k == 0:
                w = load(1)
                y[0] = (w[0], -w[1])
            back = 1 if k < 4 else 256
            if k % 4 == 0:
                ratio[2] = load(k // 2)
            for l in L1_STEPS[k]:
                y[l] = _cmul_conj(y[l - back], ratio[2])
            for q, (la, lb) in enumerate(L1):
                if lb not in L1_STEPS[k]:
                    continue
                held[q] = columns(y[la], y[lb])
                if q % 2:
                    for (to, col, a), (_, _, b) in zip(held[q - 1], held[q]):
                        b = pltpu.roll(b, 4, 0)
                        at = slice(4 * q - 4, 4 * q + 4), slice(128 * col, 128 * col + 128)
                        lhs_ref[(4 * g + 2 * to,) + at] = jnp.where(lo, a, b)
                        lhs_ref[(4 * g + 2 * to + 1,) + at] = jnp.where(lo, b, a)


def _kernel_values(g, lhs_ref, rhs_ref, tmp_ref, kd_ref):
    lane = _iota(1)
    pick = (lane & ~6) | (_iota(0) & 6)
    bit2, bit4, bit8, last = (lane & 2) != 0, (lane & 4) != 0, (lane & 8) != 0, lane == 127
    for quad in range(4):
        if quad % 2:
            yield "values"
        o = _dot_nt(_bf(lhs_ref[4 * g + quad]), _bf(rhs_ref[4 * g + quad]))
        m = [None] * 10
        for r in range(10):
            m[r ^ (quad % 2)] = jnp.take_along_axis(o[8 * r:8 * r + 8], pick, axis=1)
            if r % 4 == 1:
                yield o[8 * r:8 * r + 8]
        m = [jnp.where(bit2, m[2 * i + 1], m[2 * i]) for i in range(5)]
        for i, val in enumerate((jnp.where(bit4, m[1], m[0]), jnp.where(bit4, m[3], m[2]), m[4])):
            tmp_ref[i, 8 * quad:8 * quad + 8, :] = val
    v = [_zip(*[tmp_ref[i // 2, pl.ds(2 * c + i % 2, 8, stride=4), :] for c in range(2)]) for i in range(6)]
    v[4] = jnp.where(bit4, v[5], v[4])
    blocks = [jnp.where(bit8, pltpu.roll(v[1], 8, 1), v[0]), jnp.where(bit8, v[1], pltpu.roll(v[0], 120, 1)),
              jnp.where(last, v[1], v[2]), v[2], jnp.where(last, v[2], v[3]), v[3],
              jnp.where(last, v[3], v[4]), v[4]]
    for b in range(8):
        kd_ref[b, _rows(8 * g, 8), :] = blocks[b]


def _chunk_products(q, t, uf_ref, kf_ref, yf_ref):
    cols = slice(128 * t, 128 * t + 128)

    def load(ref, m):
        re, im = ref[m, _rows(16 * q, 8), cols], ref[m, _rows(16 * q + 8, 8), cols]
        return re, im, re + im

    prev = None
    for i0 in range(0, NC, 4):
        acc, win = [None] * 4, {}
        for m in range(i0 + 4):
            yield "conv", 6 * min(4, i0 + 4 - m) + 4
            k = load(kf_ref, m)
            for a in range(4):
                j = i0 + a - m
                if j < 0:
                    continue
                if j not in win:
                    win[j] = load(uf_ref, j)
                p = [s * u for s, u in zip(k, win[j])]
                acc[a] = p if acc[a] is None else [s + u for s, u in zip(acc[a], p)]
        for a in range(4):
            z = acc[a][0] - acc[a][1], acc[a][2] - acc[a][0] - acc[a][1]
            y = z if prev is None else (z[0] + prev[0], z[1] + prev[1])
            prev = z
            yf_ref[i0 + a, _rows(8 * q, 8), cols] = _zip(*y)


def _scores(row, qkv, prob):
    lane = _iota(1)
    even, lo64 = (lane & 32) == 0, lane < 64

    def fold(a, b, mask, shift):
        return jnp.where(mask, a, b) + pltpu.roll(jnp.where(mask, b, a), shift, 1)

    def total(terms):
        return ((terms[0] + terms[1]) + (terms[2] + terms[3])) + terms[4]

    half = []
    for pair in range(2):
        at = HALO + row + 16 * pair
        q, two = None, [None] * WIN
        for w in range(WIN // 2):
            yield "attn", 48
            q = q or [[qkv[t][_rows(at + 8 * g, 8), :] for t in range(DT)] for g in range(2)]
            k = [[qkv[DT + t][pl.ds(at - DIL * w + 8 * g, 8), :] for t in range(DT)] for g in (-1, 0, 1)]
            for far in range(2):
                first, last = [total([a * b for a, b in zip(q[g], k[g + 1 - far])]) for g in range(2)]
                x = fold(first, last, even, 32)
                two[w + 4 * far] = fold(half[0][w + 4 * far], x, lo64, 64) if pair else x
        half.append(two)
    logit = [x * (DH ** -0.5) for x in half[1]]
    if isinstance(row, int) and row < DIL * (WIN - 1):
        logit = [jnp.where(row + 8 * (lane >> 5) + _iota(0) - DIL * w >= 0, x, -1e9) for w, x in enumerate(logit)]
    yield "attn", 45
    mx = logit[0]
    for x in logit[1:]:
        mx = jnp.maximum(mx, x)
    e = [jnp.exp(x - mx) for x in logit]
    inv = 1.0 / (((e[0] + e[1]) + (e[2] + e[3])) + ((e[4] + e[5]) + (e[6] + e[7])))
    prob.extend(x * inv for x in e)


def _mix(row, o_row, qkv, prob, o_ref):
    head = _iota(1) & 31
    for pair in range(2):
        at = HALO + row + 16 * pair
        out = [None, None]
        for w in range(WIN // 2):
            yield "attn", 42
            v = [[qkv[2 * DT + t][pl.ds(at - DIL * w + 8 * g, 8), :] for t in range(DT)] for g in (-1, 0, 1)]
            for far in range(2):
                both = prob[w + 4 * far]
                for g in range(2):
                    p = jnp.take_along_axis(both, head + 32 * (2 * pair + g), axis=1)
                    terms = [p * x for x in v[g + 1 - far]]
                    out[g] = terms if out[g] is None else [s + u for s, u in zip(out[g], terms)]
        for t in range(DT):
            o_ref[_rows(o_row + 8 * pair, 8), 128 * t:128 * t + 128] = _pack(out[0][t], out[1][t])


def _interleave(slots, n_slots, work, total, gates, lead, ahead):
    done, pending, i, queue = 0, next(work, None), lead - 1, [None] * ahead
    for item in _chain(slots, [None] * ahead):
        if isinstance(item, str):
            if pending is not None and pending[2] is not None:
                gates[item](pltpu.bitcast(pending[2], jnp.int32))
            continue
        queue.append(item)
        token, gated, i = queue.pop(0), (), i + 1
        token = token() if callable(token) else token
        while pending is not None and done * n_slots < total * i:
            if token is not None and pending[0] not in gated:
                gates[pending[0]](token)
                gated = gated + (pending[0],)
            done += pending[1]
            pending = next(work, None)
    for _ in work:
        pass


def _chain(*gens):
    for g in gens:
        yield from g


def _kernel(u_hbm, are_hbm, aim_hbm, bre_hbm, bim_hbm, cre_hbm, cim_hbm, ldt_hbm, skip_hbm,
            x_hbm, w_hbm, wo_hbm, fwd_hbm, inv_hbm, out_hbm,
            ldt_ref, skip_ref, par_ref, turn_ref, direct_ref, zw_ref,
            lhs_ref, rhs_ref, tmp_ref, kd_ref,
            u_ref, w_ref, wo_ref, fwd_ref, inv_ref, xp_ref, wp_ref, wof_ref, wop_ref,
            uf_ref, kf_ref, yf_ref, qkv_ref, o_ref, ya_ref, yb_ref,
            zero_ref, isem, asem, bsem):
    zero_ref[0] = 0

    srcs = (ldt_hbm, aim_hbm, skip_hbm, are_hbm, bre_hbm, bim_hbm, cre_hbm, cim_hbm,
            u_hbm, fwd_hbm, w_hbm, x_hbm, wo_hbm, inv_hbm)
    dsts = (ldt_ref, par_ref.at[1], skip_ref, *[par_ref.at[j] for j in (0, 2, 3, 4, 5)],
            u_ref.bitcast(BF16), fwd_ref, w_ref.bitcast(BF16), xp_ref.bitcast(BF16), wo_ref.bitcast(BF16), inv_ref)
    loads = [pltpu.make_async_copy(s, d, isem.at[i]) for i, (s, d) in enumerate(zip(srcs, dsts))]

    def arrive(done, begin):
        for c in done:
            c.wait()
        for c in begin:
            c.start()

    arrive((), loads[0:2])
    arrive(loads[0:2], loads[2:9])
    dt = jnp.exp(ldt_ref[...].astype(F32)).astype(BF16).astype(F32).reshape(1, D)

    @pl.loop(0, N // 16)
    def _(i):
        rows = _rows(16 * i, 16)
        angle = dt * par_ref[1, rows, :].astype(F32)
        turn_ref[0, rows, :] = jnp.cos(angle)
        turn_ref[1, rows, :] = jnp.sin(angle)

    arrive(loads[2:8], loads[9:10])
    skip = skip_ref[...].astype(F32).reshape(1, D)
    for t in range(DT):
        cols = slice(128 * t, 128 * t + 128)
        are, bre, bim, cre, cim = [par_ref[j, :, cols].astype(F32) for j in (0, 2, 3, 4, 5)]
        h = dt[:, cols]
        e = jnp.exp(h * are)
        w = _cmul((cre, cim), (h * bre, h * bim))
        direct_ref[:, cols] = jnp.sum(w[0], axis=0, keepdims=True) + skip[:, cols]
        vals = e * turn_ref[0, :, cols], e * turn_ref[1, :, cols], w[0], w[1]
        for part in range(2):
            tr = [(v[0:128] if part == 0 else
                   jnp.concatenate([v[128:N], pltpu.roll(v[128:N], 120, 1)], axis=0)).T for v in vals]
            for r in range(0, 128, 8 + 8 * part):
                row = [v[r:r + 8] for v in tr]
                for a, v in enumerate(row + _multipliers(row[:2])):
                    zw_ref[a, part, 128 * t + r:128 * t + r + 8, :] = v

    def permute_weights():
        lane = _iota(1)
        res = lane - 5 * ((lane * 205) >> 10)
        for t in range(DT):
            idx = (DH * (lane & 31) + 5 * (lane >> 5) + t) & 127
            for r in range(D // 16):
                for p in range(3):
                    acc = None
                    for s in range(DT):
                        c0 = D * p + 128 * s
                        x = w_ref[8 * r:8 * r + 8, c0:c0 + 128]
                        acc = x if acc is None else jnp.where(res == (t - 3 * s) % 5, x, acc)
                    c0 = D * p + 128 * t
                    wp_ref[8 * r:8 * r + 8, c0:c0 + 128] = jnp.take_along_axis(acc, idx, axis=1)

    def permute_out_weights(t, cols):
        wof_ref[t] = wo_ref[:, cols]
        for dh in range(DH):
            at = 64 * (dh % 5) + 16 * (dh // 5)
            even, odd = [wof_ref[t, pl.ds(dh // 2 + DH // 2 * e, H // 2, stride=DH), :] for e in range(2)]
            if dh % 2:
                wop_ref[at:at + 16, cols] = lax.shift_right_logical(even, 16) | (odd & -65536)
            else:
                wop_ref[at:at + 16, cols] = (even & 65535) | (odd << 16)

    def transform_u(m):
        for t in range(DT):
            cols = slice(128 * t, 128 * t + 128)
            r = _dot(_bf(fwd_ref[m & 3]), _bf(u_ref[_rows(C // 2 * m, C // 2), cols]))
            uf_ref[m, 0:2 * C, cols] = r
            for i in range(0, 2 * C, 128):
                yield r[i:i + 8]

    def kernel_step(values, tables, chunk=None):
        spare = _rows(zero_ref[0], 8)

        def gate(token):
            zw_ref[14, 0, spare, :] = token

        def gate_values(token):
            rhs_ref[D // 4, spare, 0:128] = token

        slots = [_kernel_values(g, lhs_ref, rhs_ref, tmp_ref.at[j], kd_ref) for j, g in enumerate(values)]
        if chunk is not None:
            slots.append(transform_u(chunk))
        work = [_factor_tables(g, zw_ref, lhs_ref, rhs_ref) for g in tables]
        _interleave(_chain(*slots), 52, _chain(*work), 1200 * len(tables),
                    {"table": gate, "values": gate_values}, 1, 24)

    kernel_step((), (0, 1))

    @pl.loop(0, 3)
    def _(i):
        kernel_step((2 * i, 2 * i + 1), (2 * i + 2, 2 * i + 3))

    arrive(loads[8:10], loads[10:14])

    @pl.loop(3, D // 32 - 1)
    def _(i):
        kernel_step((2 * i, 2 * i + 1), (2 * i + 2, 2 * i + 3), i - 3)

    arrive(loads[10:14], ())
    permute_weights()
    for t in range(DT):
        cols = slice(128 * t, 128 * t + 128)
        if t == 1:
            kernel_step((D // 16 - 2, D // 16 - 1), ())
        for m in range(NC):
            kf_ref[m, 0:2 * C, cols] = _dot_nt(_bf(fwd_ref[m + 4]), _bf(kd_ref[CHUNK_BLOCK[m], 64 * t:64 * t + 64, :]))
        permute_out_weights(t, cols)

    def block_rows(b):
        return _rows(RB * b, RB)

    def a_copy(b):
        return pltpu.make_async_copy(ya_ref.at[block_rows(b)], out_hbm.at[block_rows(b), pl.ds(0, D)], asem.at[b])

    def b_copy(b):
        return pltpu.make_async_copy(yb_ref.at[block_rows(b)], out_hbm.at[block_rows(b), pl.ds(D, D)], bsem.at[b])

    qkv = [qkv_ref.at[c] for c in range(3 * DT)]

    def project(b):
        for c in range(3 * DT):
            r = _dot(_bf(xp_ref[_rows(RB // 2 * b, RB // 2), :]), _bf(wp_ref[:, 128 * c:128 * c + 128]))
            for i in range(0, RB, 16):
                def piece(c=c, i=i, r=r):
                    qkv[c][_rows(HALO + RB * b + i, 16), :] = r[i:i + 16]
                    return r[i + 8:i + 16]
                yield piece

    def out_project(b):
        for t in range(DT):
            cols = slice(128 * t, 128 * t + 128)
            r = _dot(_bf(o_ref[_rows(RB // 2 * b, RB // 2), :]), _bf(wop_ref[:, cols]))
            yb_ref[block_rows(b), cols] = r.astype(BF16)
            for i in range(0, RB, 16):
                yield r[i + 8:i + 16]

    def inverse(b):
        for t in range(DT):
            cols = slice(128 * t, 128 * t + 128)
            r = _dot(_bf(inv_ref[b & 3]), _bf(yf_ref[b, :, cols]))
            u = _bf(u_ref[_rows(C // 2 * b, C // 2), cols]).astype(F32)
            ya_ref[block_rows(b), cols] = (r + u * direct_ref[:, cols]).astype(BF16)
            for i in range(0, RB, 48):
                yield r[i:i + 8]

    def vector_work(columns, b_attn):
        conv = _chain(*[_chunk_products(q, t, uf_ref, kf_ref, yf_ref) for q, t in columns])
        prob = [[] for _ in range(4)]
        for g in range(5 * (b_attn is not None)):
            for _, item in zip(range(len(columns) * (8 if g else 5)), conv):
                yield item
            parts = []
            if g > 0:
                parts.append(_mix(RB * b_attn + 32 * g - 32, RB // 2 * b_attn + 16 * g - 16, qkv, prob[g - 1], o_ref))
            if g < 4:
                parts.insert(len(parts) if columns else 0, _scores(RB * b_attn + 32 * g, qkv, prob[g]))
            yield from _chain(*parts)
        yield from conv

    def step(slots, n_slots, *work):
        spare = _rows(zero_ref[0], 8)

        def gate_conv(token):
            kf_ref[NC, spare, 0:128] = token

        def gate_attn(token):
            qkv_ref[3 * DT, spare, :] = token

        total = sum(len(columns) * 976 + (b is not None) * 4 * 765 for columns, b in work)
        _interleave(slots, n_slots, _chain(*[vector_work(*w) for w in work]), total,
                    {"conv": gate_conv, "attn": gate_attn}, 10, 1)

    def region(f):
        pl.when(zero_ref[0] == 0)(f)

    def then(slots, action):
        yield from slots
        yield action

    def fill_halo():
        for c in range(DT, 3 * DT):
            qkv[c][0:HALO, :] = jnp.broadcast_to(qkv[c][HALO:HALO + 1, :], (HALO, 128))

    def inverses(blocks):
        return _chain(*[then(inverse(b), a_copy(b).start) for b in blocks])

    def outputs(b):
        return then(out_project(b), b_copy(b).start)

    columns = [(q, t) for q in range(NC) for t in range(DT)]
    region(lambda: step(_chain(then(project(0), fill_halo), project(1)), 244, (columns[:6], None), (columns[6:10], 0)))

    for b in range(2, NB, 2):
        @region
        def _():
            step(_chain(out_project(b - 2), project(b), project(b + 1), out_project(b - 1)), 325,
                 (columns[DT * b:DT * b + DT], b - 1), (columns[DT * b + DT:DT * b + 2 * DT], b))
            arrive((), [b_copy(b - 2), b_copy(b - 1)])

    step(_chain(inverses(range(0, 7)), outputs(NB - 2), inverses(range(7, 13)), outputs(NB - 1),
                inverses(range(13, NC))), 205, ([], NB - 1))
    for b in range(NB):
        a_copy(b).wait()
        b_copy(b).wait()


@jax.jit
def pallas_concat_heads__ssm_conv_s4__sliding_local_dilated__prompt_kernel(
    A_u: jax.Array,
    A_A_re: jax.Array,
    A_A_im: jax.Array,
    A_B_re: jax.Array,
    A_B_im: jax.Array,
    A_C_re: jax.Array,
    A_C_im: jax.Array,
    A_log_dt: jax.Array,
    A_Dskip: jax.Array,
    B_x: jax.Array,
    B_wqkv: jax.Array,
    B_wo: jax.Array,
):
    hbm = pl.BlockSpec(memory_space=pl.ANY)
    V = pltpu.VMEM
    I32 = jnp.int32
    scratch = [
        V((D,), BF16), V((D,), BF16), V((6, N, D), BF16),
        V((2, N, D), F32), V((1, D), F32), V((15, 2, D, 128), F32),
        V((D // 4, 40, 2 * N), I32), V((D // 4 + 1, 64, 2 * N), I32),
        V((2, 3, 32, 128), F32), V((8, D // 2, 128), I32),
        V((L // 2, D), I32), V((D // 2, 3 * D), I32), V((D // 2, D), I32),
        V(_FWD.shape, I32), V(_INV.shape, I32), V((L // 2, D), I32),
        V((D // 2, 3 * D), I32), V((DT, D // 2, 128), I32), V((D // 2, D), I32),
        V((NC, 2 * C + 8, D), F32), V((NC + 1, 2 * C + 24, D), F32), V((NC, C, D), I32),
        V((3 * DT + 1, HALO + L + 8, 128), F32), V((L // 2, D), I32),
        V((L, D), BF16), V((L, D), BF16), pltpu.SMEM((1,), I32),
        pltpu.SemaphoreType.DMA((14,)), pltpu.SemaphoreType.DMA((NB,)), pltpu.SemaphoreType.DMA((NB,)),
    ]
    out = pl.pallas_call(
        _kernel,
        out_shape=jax.ShapeDtypeStruct((L, 2 * D), BF16),
        in_specs=[hbm] * 14,
        out_specs=hbm,
        scratch_shapes=scratch,
        compiler_params=pltpu.CompilerParams(vmem_limit_bytes=120 * 1024 * 1024),
    )(A_u.reshape(L, D), A_A_re.T, A_A_im.T, A_B_re.T, A_B_im.T, A_C_re.T, A_C_im.T,
      A_log_dt, A_Dskip, B_x.reshape(L, D), B_wqkv, B_wo, _FWD, _INV)
    return out.reshape(1, L, 2 * D)
```

```python
import jax
import jax.numpy as jnp
import numpy as np
from jax import lax
import jax.experimental.pallas as pl
import jax.experimental.pallas.tpu as pltpu

L = 2048
D = 640
N = 192
H, DH = 32, 20
WIN, DIL = 8, 2
C = 128
NC = L // C
DT = D // 128
RB = 128
NB = L // RB
HALO = 16
EARLY = 6
F32 = jnp.float32
BF16 = jnp.bfloat16

L1 = ((1, 5), (2, 6), (3, 7), (4, 8), (258, 516), (260, 520), (262, 772), (264, 776), (1032, 1288), (1544, 1800))
L1_STEPS = ((1, 2), (3, 4), (5, 6), (7, 8), (258, 260, 262), (264, 516, 520), (772, 776, 1032), (1288, 1544, 1800))
CHUNK_BLOCK = (0, 1, 2, 3, 4, 5, 5, 5, 6, 7, 7, 7, 7, 7, 7, 7)


def _round_bf16(l):
    if l < 256:
        return l
    s = 1 << (l.bit_length() - 8)
    q, r = divmod(l, s)
    if 2 * r > s or (2 * r == s and q % 2 == 1):
        q += 1
    return q * s


def _row_pairs(a):
    bits = a.astype(BF16).view(np.uint16).astype(np.uint32)
    return (bits[..., 0::2, :] | (bits[..., 1::2, :] << 16)).view(np.int32)


def _dft_tables():
    row = np.arange(2 * C)
    part = (row // 8) % 2
    theta = 2.0 * np.pi * (8 * (row // 16) + row % 8 + 0.5) / (2 * C)

    def fwd(j):
        a = theta[:, None] * np.asarray(j, np.float64)[None, :]
        return np.where(part[:, None] == 0, np.cos(a), -np.sin(a))

    fu = np.stack([fwd(C * m + np.arange(C)) for m in range(4)])
    lane = np.arange(128)
    h, p, j = (lane // 8) % 2, (lane // 2) % 4, 2 * (lane // 16) + lane % 2
    l1 = np.asarray(L1)
    v = [l1[4 * (i // 2) + p, i % 2] + 8 * (16 * h + j) for i in range(4)] + [l1[8 + p % 2, p // 2] + 8 * (16 * h + j)]
    last = lane == 127
    blocks = [l1[p, h] + 8 * j, l1[p, h] + 8 * (16 + j),
              np.where(last, v[1], v[2]), v[2], np.where(last, v[2], v[3]), v[3],
              np.where(last, v[3], v[4]), v[4]]
    fk = np.zeros((NC, 2 * C, 128))
    for m in range(NC):
        for l in range(C * m + 1, min(C * m + C, L - 1) + 1):
            at = np.nonzero(blocks[CHUNK_BLOCK[m]] == _round_bf16(l))[0][0]
            fk[m, :, at] += fwd([l])[:, 0]
    inv = fu[:, 16 * (row // 16) + 8 * (row % 2) + (row // 2) % 8].transpose(0, 2, 1) / C
    return _row_pairs(fu), _row_pairs(fk), _row_pairs(inv)


_FWD_U, _FWD_K, _INV = _dft_tables()


def _iota(dim, shape=(8, 128)):
    return lax.broadcasted_iota(jnp.int32, shape, dim)


def _rows(start, size):
    return pl.ds(start if isinstance(start, int) else pl.multiple_of(start, min(size, 16)), size)


def _cmul(a, b):
    return a[0] * b[0] - a[1] * b[1], a[0] * b[1] + a[1] * b[0]


def _cmul_conj(a, b):
    return a[0] * b[0] + a[1] * b[1], a[1] * b[0] - a[0] * b[1]


def _csqr(a):
    t = a[0] * a[1]
    return a[0] * a[0] - a[1] * a[1], t + t


def _pack(a, b):
    return pltpu.bitcast(jnp.concatenate([a, b], axis=0).astype(BF16), jnp.int32)


def _zip(a, b):
    return lax.bitcast_convert_type(pltpu.pack_elementwise([a, b], packed_dtype=BF16), jnp.int32)


def _bf(a):
    return pltpu.bitcast(a, BF16)


def _dot(a, b):
    return jnp.dot(a, b, preferred_element_type=F32)


def _dot_nt(a, b):
    return lax.dot_general(a, b, (((1,), (1,)), ((), ())), preferred_element_type=F32)


def _multipliers(z1):
    lo = _iota(0) < 4
    z = {1: z1}
    for s in range(8):
        z[2 << s] = _csqr(z[1 << s])
    z8r = [pltpu.roll(t, 4, 0) for t in z[8]]
    out = list(z[256])
    for half, top in enumerate(([pltpu.roll(t, 4, 0) for t in z[128]], z[128])):
        out += [jnp.where(lo, a, b) if half == 0 else jnp.where(lo, b, a) for a, b in zip(z[8], z8r)]
        out += [jnp.where(lo, 1.0, top[0]), jnp.where(lo, 0.0, top[1])]
    return out


def _factor_tables(g, zw_ref, lhs_ref, rhs_ref):
    lo64, lo = _iota(1) < 64, _iota(0) < 4
    for part, grp in ((0, 0), (0, 1), (1, 0)):
        def load(a):
            return [zw_ref[2 * a + c, part, _rows(16 * g + 8 * grp, 8), :] for c in range(2)]

        def columns(a, b):
            re, im = _zip(a[0], b[0]), _zip(a[1], b[1])
            if part == 0:
                return (grp, 0, re), (grp, 1, im)
            return ((0, 2, jnp.where(lo64, re, pltpu.roll(im, 64, 1))),
                    (1, 2, jnp.where(lo64, pltpu.roll(re, 64, 1), im)))

        x, y, held, ratio = [None, None], {}, {}, {}
        for k in range(8):
            yield "table", (48 if part == 0 else 54), x[1] and x[1][0]
            for half in range(2):
                if k == 0 or half == 1:
                    ratio[half] = load(3 + 2 * half)
                even = load(4 + 2 * half) if k == 0 else _cmul(x[half], ratio[half])
                x[half] = _cmul(even, ratio[half])
                for to, col, val in columns(even, x[half]):
                    rhs_ref[4 * g + 2 * to + half, 8 * k:8 * k + 8, 128 * col:128 * col + 128] = val
            if k == 0:
                w = load(1)
                y[0] = (w[0], -w[1])
            back = 1 if k < 4 else 256
            if k % 4 == 0:
                ratio[2] = load(k // 2)
            for l in L1_STEPS[k]:
                y[l] = _cmul_conj(y[l - back], ratio[2])
            for q, (la, lb) in enumerate(L1):
                if lb not in L1_STEPS[k]:
                    continue
                held[q] = columns(y[la], y[lb])
                if q % 2:
                    for (to, col, a), (_, _, b) in zip(held[q - 1], held[q]):
                        b = pltpu.roll(b, 4, 0)
                        at = slice(4 * q - 4, 4 * q + 4), slice(128 * col, 128 * col + 128)
                        lhs_ref[(4 * g + 2 * to,) + at] = jnp.where(lo, a, b)
                        lhs_ref[(4 * g + 2 * to + 1,) + at] = jnp.where(lo, b, a)


def _kernel_values(g, lhs_ref, rhs_ref, tmp_ref, kd_ref):
    lane = _iota(1)
    pick = (lane & ~6) | (_iota(0) & 6)
    bit2, bit4, bit8, last = (lane & 2) != 0, (lane & 4) != 0, (lane & 8) != 0, lane == 127
    for quad in range(4):
        if quad % 2:
            yield "values"
        o = _dot_nt(_bf(lhs_ref[4 * g + quad]), _bf(rhs_ref[4 * g + quad]))
        m = [None] * 10
        for r in range(10):
            m[r ^ (quad % 2)] = jnp.take_along_axis(o[8 * r:8 * r + 8], pick, axis=1)
            if r % 4 == 1:
                yield o[8 * r:8 * r + 8]
        m = [jnp.where(bit2, m[2 * i + 1], m[2 * i]) for i in range(5)]
        for i, val in enumerate((jnp.where(bit4, m[1], m[0]), jnp.where(bit4, m[3], m[2]), m[4])):
            tmp_ref[i, 8 * quad:8 * quad + 8, :] = val
    v = [_zip(*[tmp_ref[i // 2, pl.ds(2 * c + i % 2, 8, stride=4), :] for c in range(2)]) for i in range(6)]
    v[4] = jnp.where(bit4, v[5], v[4])
    blocks = [jnp.where(bit8, pltpu.roll(v[1], 8, 1), v[0]), jnp.where(bit8, v[1], pltpu.roll(v[0], 120, 1)),
              jnp.where(last, v[1], v[2]), v[2], jnp.where(last, v[2], v[3]), v[3],
              jnp.where(last, v[3], v[4]), v[4]]
    for b in range(8):
        kd_ref[b, _rows(8 * g, 8), :] = blocks[b]


def _chunk_products(q, t, uf_ref, kf_ref, yf_ref):
    cols = slice(128 * t, 128 * t + 128)

    def load(ref, m):
        re, im = ref[m, _rows(16 * q, 8), cols], ref[m, _rows(16 * q + 8, 8), cols]
        return re, im, re + im

    prev = None
    for i0 in range(0, NC, 4):
        acc, win = [None] * 4, {}
        for m in range(i0 + 4):
            yield "conv", 6 * min(4, i0 + 4 - m) + 4
            k = load(kf_ref, m)
            for a in range(4):
                j = i0 + a - m
                if j < 0:
                    continue
                if j not in win:
                    win[j] = load(uf_ref, j)
                p = [s * u for s, u in zip(k, win[j])]
                acc[a] = p if acc[a] is None else [s + u for s, u in zip(acc[a], p)]
        for a in range(4):
            z = acc[a][0] - acc[a][1], acc[a][2] - acc[a][0] - acc[a][1]
            y = z if prev is None else (z[0] + prev[0], z[1] + prev[1])
            prev = z
            yf_ref[i0 + a, _rows(8 * q, 8), cols] = _zip(*y)


def _scores(row, qkv, prob):
    lane = _iota(1)
    even, lo64 = (lane & 32) == 0, lane < 64

    def fold(a, b, mask, shift):
        return jnp.where(mask, a, b) + pltpu.roll(jnp.where(mask, b, a), shift, 1)

    def total(terms):
        return ((terms[0] + terms[1]) + (terms[2] + terms[3])) + terms[4]

    half = []
    for pair in range(2):
        at = HALO + row + 16 * pair
        q, two = None, [None] * WIN
        for w in range(WIN // 2):
            yield "attn", 48
            q = q or [[qkv[t][_rows(at + 8 * g, 8), :] for t in range(DT)] for g in range(2)]
            k = [[qkv[DT + t][pl.ds(at - DIL * w + 8 * g, 8), :] for t in range(DT)] for g in (-1, 0, 1)]
            for far in range(2):
                first, last = [total([a * b for a, b in zip(q[g], k[g + 1 - far])]) for g in range(2)]
                x = fold(first, last, even, 32)
                two[w + 4 * far] = fold(half[0][w + 4 * far], x, lo64, 64) if pair else x
        half.append(two)
    logit = [x * (DH ** -0.5) for x in half[1]]
    if isinstance(row, int) and row < DIL * (WIN - 1):
        logit = [jnp.where(row + 8 * (lane >> 5) + _iota(0) - DIL * w >= 0, x, -1e9) for w, x in enumerate(logit)]
    yield "attn", 45
    mx = logit[0]
    for x in logit[1:]:
        mx = jnp.maximum(mx, x)
    e = [jnp.exp(x - mx) for x in logit]
    inv = 1.0 / (((e[0] + e[1]) + (e[2] + e[3])) + ((e[4] + e[5]) + (e[6] + e[7])))
    prob.extend(x * inv for x in e)


def _mix(row, o_row, qkv, prob, o_ref):
    head = _iota(1) & 31
    for pair in range(2):
        at = HALO + row + 16 * pair
        out = [None, None]
        for w in range(WIN // 2):
            yield "attn", 42
            v = [[qkv[2 * DT + t][pl.ds(at - DIL * w + 8 * g, 8), :] for t in range(DT)] for g in (-1, 0, 1)]
            for far in range(2):
                both = prob[w + 4 * far]
                for g in range(2):
                    p = jnp.take_along_axis(both, head + 32 * (2 * pair + g), axis=1)
                    terms = [p * x for x in v[g + 1 - far]]
                    out[g] = terms if out[g] is None else [s + u for s, u in zip(out[g], terms)]
        for t in range(DT):
            o_ref[_rows(o_row + 8 * pair, 8), 128 * t:128 * t + 128] = _pack(out[0][t], out[1][t])


def _interleave(slots, n_slots, work, total, gates, lead, ahead):
    done, pending, i, queue = 0, next(work, None), lead - 1, [None] * ahead
    for item in _chain(slots, [None] * ahead):
        if isinstance(item, str):
            if pending is not None and pending[2] is not None:
                gates[item](pltpu.bitcast(pending[2], jnp.int32))
            continue
        queue.append(item)
        token, gated, i = queue.pop(0), (), i + 1
        token = token() if callable(token) else token
        while pending is not None and done * n_slots < total * i:
            if token is not None and pending[0] not in gated:
                gates[pending[0]](token)
                gated = gated + (pending[0],)
            done += pending[1]
            pending = next(work, None)
    for _ in work:
        pass


def _chain(*gens):
    for g in gens:
        yield from g


def _kernel(u_hbm, are_hbm, aim_hbm, bre_hbm, bim_hbm, cre_hbm, cim_hbm, ldt_hbm, skip_hbm,
            x_hbm, w_hbm, wo_hbm, fu_hbm, fk_hbm, inv_hbm, out_hbm,
            ldt_ref, skip_ref, par_ref, aim0_ref, aim1_ref, turn_ref, direct_ref, zw_ref,
            lhs_ref, rhs_ref, tmp_ref, kd_ref,
            u0_ref, u1_ref, w_ref, wo_ref, fu_ref, fk_ref, inv_ref, x_ref, wp_ref, wof_ref, wop_ref,
            uf_ref, kf_ref, yf_ref, qkv_ref, o_ref, ya_ref, yb_ref,
            zero_ref, isem, asem, bsem):
    zero_ref[0] = 0

    pairs = (
        (ldt_hbm, ldt_ref), (aim_hbm.at[0:N // 3], aim0_ref), (aim_hbm.at[N // 3:], aim1_ref),
        (skip_hbm, skip_ref), (are_hbm, par_ref.at[0]), (bre_hbm, par_ref.at[1]), (bim_hbm, par_ref.at[2]),
        (cre_hbm, par_ref.at[3]), (cim_hbm, par_ref.at[4]),
        (u_hbm.at[0:C * EARLY], u0_ref.bitcast(BF16)), (fu_hbm, fu_ref),
        (u_hbm.at[C * EARLY:], u1_ref.bitcast(BF16)), (fk_hbm, fk_ref),
        (w_hbm, w_ref.bitcast(BF16)), (x_hbm, x_ref.bitcast(BF16)), (wo_hbm, wo_ref.bitcast(BF16)), (inv_hbm, inv_ref))
    loads = [pltpu.make_async_copy(s, d, isem.at[i]) for i, (s, d) in enumerate(pairs)]

    def region(f):
        pl.when(zero_ref[0] == 0)(f)

    def arrive(done, begin):
        for c in done:
            c.wait()
        for c in begin:
            c.start()

    arrive((), loads[0:3])
    arrive(loads[0:2], ())
    dt = jnp.exp(ldt_ref[...].astype(F32)).astype(BF16).astype(F32).reshape(1, D)

    def rotate(ref, first):
        @pl.loop(0, ref.shape[0] // 16)
        def _(i):
            angle = dt * ref[_rows(16 * i, 16), :].astype(F32)
            turn_ref[0, _rows(first + 16 * i, 16), :] = jnp.cos(angle)
            turn_ref[1, _rows(first + 16 * i, 16), :] = jnp.sin(angle)

    arrive((), loads[3:11])
    rotate(aim0_ref, 0)
    arrive(loads[2:3], ())
    rotate(aim1_ref, N // 3)
    arrive(loads[3:9], loads[11:12])

    def transform_u(m, ref, first):
        for t in range(DT):
            cols = slice(128 * t, 128 * t + 128)
            r = _dot(_bf(fu_ref[m & 3]), _bf(ref[_rows(C // 2 * (m - first), C // 2), cols]))
            uf_ref[m, 0:2 * C, cols] = r
            for i in range(0, 2 * C, 128):
                yield r[i:i + 8]

    skip = skip_ref[...].astype(F32).reshape(1, D)
    for t in range(DT):
        if t == 2:
            arrive(loads[9:11], ())
            for _ in _chain(*[transform_u(m, u0_ref, 0) for m in range(EARLY - 1)]):
                pass
        cols = slice(128 * t, 128 * t + 128)
        are, bre, bim, cre, cim = [par_ref[j, :, cols].astype(F32) for j in range(5)]
        h = dt[:, cols]
        e = jnp.exp(h * are)
        w = _cmul((cre, cim), (h * bre, h * bim))
        direct_ref[:, cols] = jnp.sum(w[0], axis=0, keepdims=True) + skip[:, cols]
        vals = e * turn_ref[0, :, cols], e * turn_ref[1, :, cols], w[0], w[1]
        for part in range(2):
            tr = [(v[0:128] if part == 0 else
                   jnp.concatenate([v[128:N], pltpu.roll(v[128:N], 120, 1)], axis=0)).T for v in vals]
            for r in range(0, 128, 8 + 8 * part):
                row = [v[r:r + 8] for v in tr]
                for a, v in enumerate(row + _multipliers(row[:2])):
                    zw_ref[a, part, 128 * t + r:128 * t + r + 8, :] = v

    def permute_weights():
        lane = _iota(1)
        res = lane - 5 * ((lane * 205) >> 10)
        for t in range(DT):
            idx = (DH * (lane & 31) + 5 * (lane >> 5) + t) & 127
            for r in range(D // 16):
                for p in range(3):
                    acc = None
                    for s in range(DT):
                        c0 = D * p + 128 * s
                        x = w_ref[8 * r:8 * r + 8, c0:c0 + 128]
                        acc = x if acc is None else jnp.where(res == (t - 3 * s) % 5, x, acc)
                    c0 = D * p + 128 * t
                    wp_ref[8 * r:8 * r + 8, c0:c0 + 128] = jnp.take_along_axis(acc, idx, axis=1)

    def permute_out_weights(t, cols):
        wof_ref[t] = wo_ref[:, cols]
        for dh in range(DH):
            at = 64 * (dh % 5) + 16 * (dh // 5)
            even, odd = [wof_ref[t, pl.ds(dh // 2 + DH // 2 * e, H // 2, stride=DH), :] for e in range(2)]
            if dh % 2:
                wop_ref[at:at + 16, cols] = lax.shift_right_logical(even, 16) | (odd & -65536)
            else:
                wop_ref[at:at + 16, cols] = (even & 65535) | (odd << 16)

    def transform_k(tiles):
        for t, m in tiles:
            r = _dot_nt(_bf(fk_ref[m]), _bf(kd_ref[CHUNK_BLOCK[m], _rows(64 * t, 64), :]))
            kf_ref[m, 0:2 * C, 128 * t:128 * t + 128] = r
            for i in range(0, 2 * C, 128):
                yield r[i:i + 8]

    def kernel_step(values, tables, transform=()):
        spare = _rows(zero_ref[0], 8)

        def gate(token):
            zw_ref[14, 0, spare, :] = token

        def gate_values(token):
            rhs_ref[D // 4, spare, 0:128] = token

        slots = [_kernel_values(g, lhs_ref, rhs_ref, tmp_ref.at[j], kd_ref) for j, g in enumerate(values)]
        work = [_factor_tables(g, zw_ref, lhs_ref, rhs_ref) for g in tables]
        _interleave(_chain(*slots, transform), 52, _chain(*work), 1200 * len(tables),
                    {"table": gate, "values": gate_values}, 1, 24)

    region(lambda: kernel_step((), (0, 1)))


    region(lambda: kernel_step((0, 1), (2, 3), transform_u(EARLY - 1, u0_ref, 0)))
    arrive(loads[11:12], loads[12:17])

    @pl.loop(1, NC - EARLY + 1)
    def _(i):
        kernel_step((2 * i, 2 * i + 1), (2 * i + 2, 2 * i + 3), transform_u(i + EARLY - 1, u1_ref, EARLY))

    arrive(loads[12:13], ())
    todo = [(t, m) for t in range(DT) for m in range(NC)]
    for i in range(NC - EARLY + 1, D // 32 - 1):
        region(lambda: kernel_step((2 * i, 2 * i + 1), (2 * i + 2, 2 * i + 3), transform_k(todo[:5])))
        todo = todo[5:]

    arrive(loads[13:17], ())
    permute_weights()
    for _ in transform_k(todo[:8]):
        pass
    kernel_step((D // 16 - 2, D // 16 - 1), ())
    for _ in transform_k(todo[8:]):
        pass
    for t in range(DT):
        permute_out_weights(t, slice(128 * t, 128 * t + 128))

    def block_rows(b):
        return _rows(RB * b, RB)

    def a_copy(b):
        return pltpu.make_async_copy(ya_ref.at[block_rows(b)], out_hbm.at[block_rows(b), pl.ds(0, D)], asem.at[b])

    def b_copy(b):
        return pltpu.make_async_copy(yb_ref.at[block_rows(b)], out_hbm.at[block_rows(b), pl.ds(D, D)], bsem.at[b])

    qkv = [qkv_ref.at[c] for c in range(3 * DT)]

    def project(b):
        for c in range(3 * DT):
            r = _dot(_bf(x_ref[_rows(RB // 2 * b, RB // 2), :]), _bf(wp_ref[:, 128 * c:128 * c + 128]))
            for i in range(0, RB, 16):
                def piece(c=c, i=i, r=r):
                    qkv[c][_rows(HALO + RB * b + i, 16), :] = r[i:i + 16]
                    return r[i + 8:i + 16]
                yield piece

    def out_project(b):
        for t in range(DT):
            cols = slice(128 * t, 128 * t + 128)
            r = _dot(_bf(o_ref[_rows(RB // 2 * b, RB // 2), :]), _bf(wop_ref[:, cols]))
            yb_ref[block_rows(b), cols] = r.astype(BF16)
            for i in range(0, RB, 16):
                yield r[i + 8:i + 16]

    def inverse(b):
        for t in range(DT):
            cols = slice(128 * t, 128 * t + 128)
            r = _dot(_bf(inv_ref[b & 3]), _bf(yf_ref[b, :, cols]))
            ref, first = (u0_ref, 0) if b < EARLY else (u1_ref, EARLY)
            u = _bf(ref[_rows(C // 2 * (b - first), C // 2), cols]).astype(F32)
            ya_ref[block_rows(b), cols] = (r + u * direct_ref[:, cols]).astype(BF16)
            for i in range(0, RB, 48):
                yield r[i:i + 8]

    def vector_work(columns, b_attn):
        conv = _chain(*[_chunk_products(q, t, uf_ref, kf_ref, yf_ref) for q, t in columns])
        prob = [[] for _ in range(4)]
        for g in range(5 * (b_attn is not None)):
            for _, item in zip(range(len(columns) * (8 if g else 5)), conv):
                yield item
            parts = []
            if g > 0:
                parts.append(_mix(RB * b_attn + 32 * g - 32, RB // 2 * b_attn + 16 * g - 16, qkv, prob[g - 1], o_ref))
            if g < 4:
                parts.insert(len(parts) if columns else 0, _scores(RB * b_attn + 32 * g, qkv, prob[g]))
            yield from _chain(*parts)
        yield from conv

    def step(slots, n_slots, *work):
        spare = _rows(zero_ref[0], 8)

        def gate_conv(token):
            kf_ref[NC, spare, 0:128] = token

        def gate_attn(token):
            qkv_ref[3 * DT, spare, :] = token

        total = sum(len(columns) * 976 + (b is not None) * 4 * 765 for columns, b in work)
        _interleave(slots, n_slots, _chain(*[vector_work(*w) for w in work]), total,
                    {"conv": gate_conv, "attn": gate_attn}, 10, 1)

    def then(slots, action):
        yield from slots
        yield action

    def fill_halo():
        for c in range(DT, 3 * DT):
            qkv[c][0:HALO, :] = jnp.broadcast_to(qkv[c][HALO:HALO + 1, :], (HALO, 128))

    def inverses(blocks):
        return _chain(*[then(inverse(b), a_copy(b).start) for b in blocks])

    def outputs(b):
        return then(out_project(b), b_copy(b).start)

    columns = [(q, t) for q in range(NC) for t in range(DT)]
    region(lambda: step(_chain(then(project(0), fill_halo), project(1)), 244, (columns[:6], None), (columns[6:10], 0)))

    for b in range(2, NB, 2):
        @region
        def _():
            step(_chain(out_project(b - 2), project(b), project(b + 1), out_project(b - 1)), 325,
                 (columns[DT * b:DT * b + DT], b - 1), (columns[DT * b + DT:DT * b + 2 * DT], b))
            arrive((), [b_copy(b - 2), b_copy(b - 1)])

    step(_chain(inverses(range(0, 7)), outputs(NB - 2), inverses(range(7, 13)), outputs(NB - 1),
                inverses(range(13, NC))), 205, ([], NB - 1))
    for b in range(NB):
        a_copy(b).wait()
        b_copy(b).wait()


@jax.jit
def pallas_concat_heads__ssm_conv_s4__sliding_local_dilated__prompt_kernel(
    A_u: jax.Array,
    A_A_re: jax.Array,
    A_A_im: jax.Array,
    A_B_re: jax.Array,
    A_B_im: jax.Array,
    A_C_re: jax.Array,
    A_C_im: jax.Array,
    A_log_dt: jax.Array,
    A_Dskip: jax.Array,
    B_x: jax.Array,
    B_wqkv: jax.Array,
    B_wo: jax.Array,
):
    hbm = pl.BlockSpec(memory_space=pl.ANY)
    V = pltpu.VMEM
    I32 = jnp.int32
    scratch = [
        V((D,), BF16), V((D,), BF16), V((5, N, D), BF16), V((N // 3, D), BF16), V((N - N // 3, D), BF16),
        V((2, N, D), F32), V((1, D), F32), V((15, 2, D, 128), F32),
        V((D // 4, 40, 2 * N), I32), V((D // 4 + 1, 64, 2 * N), I32),
        V((2, 3, 32, 128), F32), V((8, D // 2, 128), I32),
        V((C * EARLY // 2, D), I32), V(((L - C * EARLY) // 2, D), I32), V((D // 2, 3 * D), I32), V((D // 2, D), I32),
        V(_FWD_U.shape, I32), V(_FWD_K.shape, I32), V(_INV.shape, I32), V((L // 2, D), I32),
        V((D // 2, 3 * D), I32), V((DT, D // 2, 128), I32), V((D // 2, D), I32),
        V((NC, 2 * C + 8, D), F32), V((NC + 1, 2 * C + 24, D), F32), V((NC, C, D), I32),
        V((3 * DT + 1, HALO + L + 8, 128), F32), V((L // 2, D), I32),
        V((L, D), BF16), V((L, D), BF16), pltpu.SMEM((1,), I32),
        pltpu.SemaphoreType.DMA((17,)), pltpu.SemaphoreType.DMA((NB,)), pltpu.SemaphoreType.DMA((NB,)),
    ]
    out = pl.pallas_call(
        _kernel,
        out_shape=jax.ShapeDtypeStruct((L, 2 * D), BF16),
        in_specs=[hbm] * 15,
        out_specs=hbm,
        scratch_shapes=scratch,
        compiler_params=pltpu.CompilerParams(vmem_limit_bytes=120 * 1024 * 1024),
    )(A_u.reshape(L, D), A_A_re.T, A_A_im.T, A_B_re.T, A_B_im.T, A_C_re.T, A_C_im.T,
      A_log_dt, A_Dskip, B_x.reshape(L, D), B_wqkv, B_wo, _FWD_U, _FWD_K, _INV)
    return out.reshape(1, L, 2 * D)
```
